```python
import jax
import jax.numpy as jnp

def _softmax(x, axis=-1):
    return jax.nn.softmax(x, axis=axis)
def _gelu(x):
    return jax.nn.gelu(x, approximate=True)
def _silu(x):
    return jax.nn.silu(x)
def _sigmoid(x):
    return jax.nn.sigmoid(x)
def _layernorm(x, axis=-1, eps=1e-5):
    m = jnp.mean(x, axis=axis, keepdims=True)
    v = jnp.var(x, axis=axis, keepdims=True)
    return (x - m) / jnp.sqrt(v + eps)
def _scatter_add(tgt, idx, src, axis=0):
    return tgt.at[idx].add(src)
def _segment_sum(src, seg, n):
    return jax.ops.segment_sum(src, seg, n)
class _Rng:
    def __init__(self, key):
        self._k = key
    def _next(self):
        self._k, sub = jax.random.split(self._k)
        return sub
    def normal(self, shape):
        return jax.random.normal(self._next(), shape, dtype=jnp.bfloat16)
    def randint(self, lo, hi, shape):
        return jax.random.randint(self._next(), shape, lo, hi, dtype=jnp.int32)
    def uniform(self, shape, lo=0.0, hi=1.0):
        return jax.random.uniform(self._next(), shape, jnp.bfloat16, lo, hi)
    def permutation(self, n):
        return jax.random.permutation(self._next(), n)


kernel_name = 'concat_heads__gqa_block_cached__gqa_block_cached__near_ridge'

def setup_inputs():
    _rng = _Rng(jax.random.key(int.from_bytes(__import__("os").urandom(4), "little")))
    _w = (lambda a: (lambda t: t.astype(jnp.bfloat16) if jnp.issubdtype(t.dtype, jnp.floating) else t)(jnp.asarray(a)))
    def _A_setup():
        B, Sq, D = 8, 256, 640
        Hq, Hkv, Sk, Dh = 32, 32, 1024, 192
        assert Hq % Hkv == 0, (Hq, Hkv)
        return {
            "x": _w((lambda *s: _rng.normal(s) * 0.05)(B, Sq, D)),
            "k_cache": _w((lambda *s: _rng.normal(s) * 0.05)(B, Hkv, Sk, Dh)),
            "v_cache": _w((lambda *s: _rng.normal(s) * 0.05)(B, Hkv, Sk, Dh)),
            "wq": _w((lambda *s: _rng.normal(s) * 0.05)(D, Hq * Dh) * (D ** -0.5)),
            "wo": _w((lambda *s: _rng.normal(s) * 0.05)(Hq * Dh, D) * ((Hq * Dh) ** -0.5)),
        }
    _A_in = _A_setup()

    def _B_setup():
        B, Sq, D = 8, 256, 640
        Hq, Hkv, Sk, Dh = 32, 32, 1024, 192
        assert Hq % Hkv == 0, (Hq, Hkv)
        return {
            "x": _w((lambda *s: _rng.normal(s) * 0.05)(B, Sq, D)),
            "k_cache": _w((lambda *s: _rng.normal(s) * 0.05)(B, Hkv, Sk, Dh)),
            "v_cache": _w((lambda *s: _rng.normal(s) * 0.05)(B, Hkv, Sk, Dh)),
            "wq": _w((lambda *s: _rng.normal(s) * 0.05)(D, Hq * Dh) * (D ** -0.5)),
            "wo": _w((lambda *s: _rng.normal(s) * 0.05)(Hq * Dh, D) * ((Hq * Dh) ** -0.5)),
        }
    _B_in = _B_setup()

    return {
        "A_x": _A_in["x"],
        "A_k_cache": _A_in["k_cache"],
        "A_v_cache": _A_in["v_cache"],
        "A_wq": _A_in["wq"],
        "A_wo": _A_in["wo"],
        "B_x": _B_in["x"],
        "B_k_cache": _B_in["k_cache"],
        "B_v_cache": _B_in["v_cache"],
        "B_wq": _B_in["wq"],
        "B_wo": _B_in["wo"],
    }

def reference(A_x, A_k_cache, A_v_cache, A_wq, A_wo, B_x, B_k_cache, B_v_cache, B_wq, B_wo):
    def _A_ref(x, k_cache, v_cache, wq, wo):
        B, Sq, D = x.shape
        Hq, Dh = 32, 192
        Hkv = k_cache.shape[1]
        rep = Hq // Hkv
        q = (lambda x, *d: x.transpose(*d))((x @ wq).reshape(B, Sq, Hq, Dh), 0, 2, 1, 3)
        k = jnp.repeat(k_cache, rep, axis=1)
        v = jnp.repeat(v_cache, rep, axis=1)
        scores = jnp.einsum("bhqd,bhkd->bhqk", q, k) * (Dh ** -0.5)
        p = _softmax(scores, axis=-1)
        o = jnp.einsum("bhqk,bhkd->bhqd", p, v)
        return (lambda x, *d: x.transpose(*d))(o, 0, 2, 1, 3).reshape(B, Sq, Hq * Dh) @ wo

    def _B_ref(x, k_cache, v_cache, wq, wo):
        B, Sq, D = x.shape
        Hq, Dh = 32, 192
        Hkv = k_cache.shape[1]
        rep = Hq // Hkv
        q = (lambda x, *d: x.transpose(*d))((x @ wq).reshape(B, Sq, Hq, Dh), 0, 2, 1, 3)
        k = jnp.repeat(k_cache, rep, axis=1)
        v = jnp.repeat(v_cache, rep, axis=1)
        scores = jnp.einsum("bhqd,bhkd->bhqk", q, k) * (Dh ** -0.5)
        p = _softmax(scores, axis=-1)
        o = jnp.einsum("bhqk,bhkd->bhqd", p, v)
        return (lambda x, *d: x.transpose(*d))(o, 0, 2, 1, 3).reshape(B, Sq, Hq * Dh) @ wo

    a = _A_ref(A_x, A_k_cache, A_v_cache, A_wq, A_wo)
    b = _B_ref(B_x, B_k_cache, B_v_cache, B_wq, B_wo)
    return jnp.concatenate([a, b], axis=-1)
```

```python
import functools
import math

import jax
import jax.numpy as jnp
from jax import lax
import jax.experimental.pallas as pl
import jax.experimental.pallas.tpu as pltpu

_HQ = 32
_DH = 192
_LANES = 128


def _nn(a, b):
    return lax.dot_general(a, b, (((1,), (0,)), ((), ())),
                           preferred_element_type=jnp.float32)


def _nt(a, b):
    return lax.dot_general(a, b, (((1,), (1,)), ((), ())),
                           preferred_element_type=jnp.float32)


def _tn(a, b):
    return lax.dot_general(a, b, (((0,), (0,)), ((), ())),
                           preferred_element_type=jnp.float32)


def _softmax_rows(s):
    m = jnp.max(s, axis=1, keepdims=True)
    e = jnp.exp2(s - m)
    l = jnp.sum(e, axis=1, keepdims=True)
    return (e * (1.0 / l)).astype(jnp.bfloat16)


def _pair(x, wq_ref, k_ref, v_ref, wo_ref):
    scale = (_DH ** -0.5) * math.log2(math.e)
    q = (_nn(x, wq_ref[...]) * scale).astype(jnp.bfloat16)
    lane = lax.broadcasted_iota(jnp.int32, (q.shape[0], 2 * _LANES), 1)
    q0 = jnp.where(lane < _DH, q[:, :256], 0)
    q1 = jnp.where(lane >= _DH - _LANES, q[:, 128:], 0)
    s0 = _nn(q0, k_ref[0:256, :])
    s1 = _nn(q1, k_ref[128:384, :])
    p0 = _softmax_rows(s0)
    p1 = _softmax_rows(s1)
    o0 = _nt(v_ref[0:_DH, :], p0)
    o1 = _nt(v_ref[_DH:2 * _DH, :], p1)
    ot = jnp.concatenate([o0, o1], axis=0).astype(jnp.bfloat16)
    return _tn(ot, wo_ref[...])


def _kernel(xa_ref, ka_ref, va_ref, wqa_ref, woa_ref,
            xb_ref, kb_ref, vb_ref, wqb_ref, wob_ref,
            o_ref, acc_ref, *, n_pairs, d):
    p = pl.program_id(0)
    b = pl.program_id(1)

    @pl.when(p == 0)
    def _():
        acc_ref[b] = jnp.zeros(acc_ref.shape[1:], jnp.float32)

    ra = _pair(xa_ref[b], wqa_ref, ka_ref, va_ref, woa_ref)
    rb = _pair(xb_ref[b], wqb_ref, kb_ref, vb_ref, wob_ref)
    acc_ref[b] += jnp.concatenate([ra, rb], axis=1)

    @pl.when(p == n_pairs - 1)
    def _():
        o_ref[...] = acc_ref[b].astype(o_ref.dtype)


@jax.jit
def pallas_concat_heads__gqa_block_cached__gqa_block_cached__near_ridge_kernel(
    A_x: jax.Array,
    A_k_cache: jax.Array,
    A_v_cache: jax.Array,
    A_wq: jax.Array,
    A_wo: jax.Array,
    B_x: jax.Array,
    B_k_cache: jax.Array,
    B_v_cache: jax.Array,
    B_wq: jax.Array,
    B_wo: jax.Array,
):
    B, Sq, D = A_x.shape
    Hkv, Sk, Dh = A_k_cache.shape[1:]
    assert Hkv == _HQ and Dh == _DH
    n_pairs = _HQ // 2
    W = 2 * _DH

    def kv(a):
        return jnp.swapaxes(a, 2, 3).reshape(B, _HQ * _DH, Sk)

    x_spec = pl.BlockSpec((B, Sq, D), lambda p, b: (0, 0, 0))
    kv_spec = pl.BlockSpec((None, W, Sk), lambda p, b: (b, p, 0))
    wq_spec = pl.BlockSpec((D, W), lambda p, b: (0, p))
    wo_spec = pl.BlockSpec((W, D), lambda p, b: (p, 0))
    specs = [x_spec, kv_spec, kv_spec, wq_spec, wo_spec]
    out_spec = pl.BlockSpec(
        (None, Sq, 2 * D),
        lambda p, b: (jnp.where(p == n_pairs - 1, b, 0), 0, 0))

    return pl.pallas_call(
        functools.partial(_kernel, n_pairs=n_pairs, d=D),
        grid=(n_pairs, B),
        in_specs=specs + specs,
        out_specs=out_spec,
        out_shape=jax.ShapeDtypeStruct((B, Sq, 2 * D), A_x.dtype),
        scratch_shapes=[pltpu.VMEM((B, Sq, 2 * D), jnp.float32)],
        compiler_params=pltpu.CompilerParams(
            dimension_semantics=("arbitrary", "arbitrary"),
            vmem_limit_bytes=100 * 1024 * 1024,
        ),
    )(A_x, kv(A_k_cache), kv(A_v_cache), A_wq, A_wo,
      B_x, kv(B_k_cache), kv(B_v_cache), B_wq, B_wo)
```

```python
import functools
import math

import jax
import jax.numpy as jnp
from jax import lax
import jax.experimental.pallas as pl
import jax.experimental.pallas.tpu as pltpu

_HQ = 32
_DH = 192
_LANES = 128
_NP = 2


def _nn(a, b):
    return lax.dot_general(a, b, (((1,), (0,)), ((), ())),
                           preferred_element_type=jnp.float32)


def _nt(a, b):
    return lax.dot_general(a, b, (((1,), (1,)), ((), ())),
                           preferred_element_type=jnp.float32)


def _tn(a, b):
    return lax.dot_general(a, b, (((0,), (0,)), ((), ())),
                           preferred_element_type=jnp.float32)


def _kernel(xa_ref, ka_ref, va_ref, wqa_ref, woa_ref,
            xb_ref, kb_ref, vb_ref, wqb_ref, wob_ref,
            o_ref, acc_ref, q_scr, p_scr, ot_scr, *, n_pairs, d):
    p = pl.program_id(0)
    b = pl.program_id(1)
    sq = o_ref.shape[0]

    @pl.when(p == 0)
    def _():
        acc_ref[b] = jnp.zeros(acc_ref.shape[1:], jnp.float32)

    xs = (xa_ref, xb_ref)
    wqs = (wqa_ref, wqb_ref)
    ks = (ka_ref, kb_ref)
    vs = (va_ref, vb_ref)
    wos = (woa_ref, wob_ref)
    scale = (_DH ** -0.5) * math.log2(math.e)

    items = [(i, t) for i in range(2) for t in range(_NP)]
    W = 2 * _DH

    def qproj(n):
        i, t = items[n]
        q = _nn(xs[i][...], wqs[i][:, W * t:W * (t + 1)]) * scale
        lane = lax.broadcasted_iota(jnp.int32, (sq, _LANES), 1)
        mid = q[:, 128:256]
        q_scr[n, :, 0:128] = q[:, 0:128].astype(jnp.bfloat16)
        q_scr[n, :, 128:256] = jnp.where(lane < 64, mid, 0.0).astype(jnp.bfloat16)
        q_scr[n, :, 256:384] = jnp.where(lane >= 64, mid, 0.0).astype(jnp.bfloat16)
        q_scr[n, :, 384:512] = q[:, 256:384].astype(jnp.bfloat16)

    def scores(n, h):
        i, t = items[n]
        r = W * t + 128 * h
        s = _nn(q_scr[n, :, 256 * h:256 * h + 256], ks[i][r:r + 256, :])
        m = jnp.max(s, axis=1, keepdims=True)
        p_scr[2 * n + h] = jnp.exp2(s - m).astype(jnp.bfloat16)

    def pv(n, h):
        i, t = items[n]
        r = W * t + _DH * h
        vt = vs[i][r:r + _DH, :]
        pb = p_scr[2 * n + h]
        part = pb[:, 0:128].astype(jnp.float32)
        for c in range(128, pb.shape[1], 128):
            part = part + pb[:, c:c + 128].astype(jnp.float32)
        inv = 1.0 / jnp.sum(part.T, axis=0, keepdims=True)
        o = _nt(vt, pb) * inv
        ot_scr[i, r:r + _DH, :] = o.astype(jnp.bfloat16)

    def oproj(i):
        acc_ref[b, :, d * i:d * (i + 1)] += _tn(ot_scr[i], wos[i][...])

    qproj(0)
    qproj(1)
    qproj(2)
    qproj(3)
    scores(0, 0)
    scores(0, 1)
    pv(0, 0)
    scores(1, 0)
    pv(0, 1)
    scores(1, 1)
    pv(1, 0)
    scores(2, 0)
    pv(1, 1)
    scores(2, 1)
    pv(2, 0)
    scores(3, 0)
    pv(2, 1)
    scores(3, 1)
    pv(3, 0)
    pv(3, 1)
    oproj(0)
    oproj(1)

    @pl.when(p == n_pairs - 1)
    def _():
        o_ref[...] = acc_ref[b].astype(o_ref.dtype)


@jax.jit
def pallas_concat_heads__gqa_block_cached__gqa_block_cached__near_ridge_kernel(
    A_x: jax.Array,
    A_k_cache: jax.Array,
    A_v_cache: jax.Array,
    A_wq: jax.Array,
    A_wo: jax.Array,
    B_x: jax.Array,
    B_k_cache: jax.Array,
    B_v_cache: jax.Array,
    B_wq: jax.Array,
    B_wo: jax.Array,
):
    B, Sq, D = A_x.shape
    Hkv, Sk, Dh = A_k_cache.shape[1:]
    assert Hkv == _HQ and Dh == _DH
    n_pairs = _HQ // (2 * _NP)
    W = 2 * _DH * _NP

    def kv(a):
        return jnp.swapaxes(a, 2, 3).reshape(B, _HQ * _DH, Sk)

    x_spec = pl.BlockSpec((None, Sq, D), lambda p, b: (b, 0, 0))
    kv_spec = pl.BlockSpec((None, W, Sk), lambda p, b: (b, p, 0))
    wq_spec = pl.BlockSpec((D, W), lambda p, b: (0, p))
    wo_spec = pl.BlockSpec((W, D), lambda p, b: (p, 0))
    specs = [x_spec, kv_spec, kv_spec, wq_spec, wo_spec]
    out_spec = pl.BlockSpec(
        (None, Sq, 2 * D),
        lambda p, b: (jnp.where(p == n_pairs - 1, b, 0), 0, 0))

    return pl.pallas_call(
        functools.partial(_kernel, n_pairs=n_pairs, d=D),
        grid=(n_pairs, B),
        in_specs=specs + specs,
        out_specs=out_spec,
        out_shape=jax.ShapeDtypeStruct((B, Sq, 2 * D), A_x.dtype),
        scratch_shapes=[
            pltpu.VMEM((B, Sq, 2 * D), jnp.float32),
            pltpu.VMEM((2 * _NP, Sq, 512), jnp.bfloat16),
            pltpu.VMEM((4 * _NP, Sq, Sk), jnp.bfloat16),
            pltpu.VMEM((2, W, Sq), jnp.bfloat16),
        ],
        compiler_params=pltpu.CompilerParams(
            dimension_semantics=("arbitrary", "arbitrary"),
            vmem_limit_bytes=100 * 1024 * 1024,
        ),
    )(A_x, kv(A_k_cache), kv(A_v_cache), A_wq, A_wo,
      B_x, kv(B_k_cache), kv(B_v_cache), B_wq, B_wo)
```

```python
import functools
import math

import jax
import jax.numpy as jnp
from jax import lax
import jax.experimental.pallas as pl
import jax.experimental.pallas.tpu as pltpu

_HQ = 32
_DH = 192
_LANES = 128
_NP = 2


def _nn(a, b):
    return lax.dot_general(a, b, (((1,), (0,)), ((), ())),
                           preferred_element_type=jnp.float32)


def _nt(a, b):
    return lax.dot_general(a, b, (((1,), (1,)), ((), ())),
                           preferred_element_type=jnp.float32)


def _tn(a, b):
    return lax.dot_general(a, b, (((0,), (0,)), ((), ())),
                           preferred_element_type=jnp.float32)


def _kernel(xa_ref, ka_ref, va_ref, wqa_ref, woa_ref,
            xb_ref, kb_ref, vb_ref, wqb_ref, wob_ref,
            o_ref, acc_ref, q_scr, p_scr, ot_scr, *, n_steps, d):
    p = pl.program_id(0)
    b = pl.program_id(1)
    sq = o_ref.shape[0]

    @pl.when(p == 0)
    def _():
        acc_ref[b] = jnp.zeros(acc_ref.shape[1:], jnp.float32)

    xs = (xa_ref, xb_ref)
    wqs = (wqa_ref, wqb_ref)
    ks = (ka_ref, kb_ref)
    vs = (va_ref, vb_ref)
    wos = (woa_ref, wob_ref)
    scale = (_DH ** -0.5) * math.log2(math.e)

    items = [(i, t) for i in range(2) for t in range(_NP)]
    W = 2 * _DH

    def qproj(n):
        i, t = items[n]
        q = _nn(xs[i][...], wqs[i][:, W * t:W * (t + 1)]) * scale
        lane = lax.broadcasted_iota(jnp.int32, (sq, _LANES), 1)
        mid = q[:, 128:256]
        q_scr[n, :, 0:128] = q[:, 0:128].astype(jnp.bfloat16)
        q_scr[n, :, 128:256] = jnp.where(lane < 64, mid, 0.0).astype(jnp.bfloat16)
        q_scr[n, :, 256:384] = jnp.where(lane >= 64, mid, 0.0).astype(jnp.bfloat16)
        q_scr[n, :, 384:512] = q[:, 256:384].astype(jnp.bfloat16)

    def scores(n, h):
        i, t = items[n]
        r = W * t + 128 * h
        s = _nn(q_scr[n, :, 256 * h:256 * h + 256], ks[i][r:r + 256, :])
        m = jnp.max(s, axis=1, keepdims=True)
        p_scr[2 * n + h] = jnp.exp2(s - m).astype(jnp.bfloat16)

    def pv(n, h):
        i, t = items[n]
        r = W * t + _DH * h
        vt = vs[i][r:r + _DH, :]
        pb = p_scr[2 * n + h]
        part = pb[:, 0:128].astype(jnp.float32)
        for c in range(128, pb.shape[1], 128):
            part = part + pb[:, c:c + 128].astype(jnp.float32)
        inv = 1.0 / jnp.sum(part.T, axis=0, keepdims=True)
        o = _nt(vt, pb) * inv
        ot_scr[i, r:r + _DH, :] = o.astype(jnp.bfloat16)

    def oproj(i):
        acc_ref[b, :, d * i:d * (i + 1)] += _tn(ot_scr[i], wos[i][...])

    for n in range(len(items)):
        qproj(n)
    heads = [(n, h) for n in range(len(items)) for h in range(2)]
    for j in range(len(heads) + 1):
        if j < len(heads):
            scores(*heads[j])
        if j > 0:
            pv(*heads[j - 1])
    oproj(0)
    oproj(1)

    @pl.when(p == n_steps - 1)
    def _():
        o_ref[...] = acc_ref[b].astype(o_ref.dtype)


@jax.jit
def pallas_concat_heads__gqa_block_cached__gqa_block_cached__near_ridge_kernel(
    A_x: jax.Array,
    A_k_cache: jax.Array,
    A_v_cache: jax.Array,
    A_wq: jax.Array,
    A_wo: jax.Array,
    B_x: jax.Array,
    B_k_cache: jax.Array,
    B_v_cache: jax.Array,
    B_wq: jax.Array,
    B_wo: jax.Array,
):
    B, Sq, D = A_x.shape
    Hkv, Sk, Dh = A_k_cache.shape[1:]
    assert Hkv == _HQ and Dh == _DH
    n_steps = _HQ // (2 * _NP)
    W = 2 * _DH * _NP

    def kv(a):
        return jnp.swapaxes(a, 2, 3).reshape(B, _HQ * _DH, Sk)

    x_spec = pl.BlockSpec((None, Sq, D), lambda p, b: (b, 0, 0))
    kv_spec = pl.BlockSpec((None, W, Sk), lambda p, b: (b, p, 0))
    wq_spec = pl.BlockSpec((D, W), lambda p, b: (0, p))
    wo_spec = pl.BlockSpec((W, D), lambda p, b: (p, 0))
    specs = [x_spec, kv_spec, kv_spec, wq_spec, wo_spec]
    out_spec = pl.BlockSpec(
        (None, Sq, 2 * D),
        lambda p, b: (jnp.where(p == n_steps - 1, b, 0), 0, 0))

    return pl.pallas_call(
        functools.partial(_kernel, n_steps=n_steps, d=D),
        grid=(n_steps, B),
        in_specs=specs + specs,
        out_specs=out_spec,
        out_shape=jax.ShapeDtypeStruct((B, Sq, 2 * D), A_x.dtype),
        scratch_shapes=[
            pltpu.VMEM((B, Sq, 2 * D), jnp.float32),
            pltpu.VMEM((2 * _NP, Sq, 512), jnp.bfloat16),
            pltpu.VMEM((4 * _NP, Sq, Sk), jnp.bfloat16),
            pltpu.VMEM((2, W, Sq), jnp.bfloat16),
        ],
        compiler_params=pltpu.CompilerParams(
            dimension_semantics=("arbitrary", "arbitrary"),
            vmem_limit_bytes=100 * 1024 * 1024,
        ),
    )(A_x, kv(A_k_cache), kv(A_v_cache), A_wq, A_wo,
      B_x, kv(B_k_cache), kv(B_v_cache), B_wq, B_wo)
```
